```python
import os as _os
_os.environ.setdefault("JAX_PLATFORMS", "cpu")
import jax
import jax.numpy as jnp

def _softmax(x, axis=-1):
    return jax.nn.softmax(x, axis=axis)
def _gelu(x):
    return jax.nn.gelu(x, approximate=True)
def _silu(x):
    return jax.nn.silu(x)
def _sigmoid(x):
    return jax.nn.sigmoid(x)
def _layernorm(x, axis=-1, eps=1e-5):
    m = jnp.mean(x, axis=axis, keepdims=True)
    v = jnp.var(x, axis=axis, keepdims=True)
    return (x - m) / jnp.sqrt(v + eps)
def _scatter_add(tgt, idx, src, axis=0):
    return tgt.at[idx].add(src)
def _segment_sum(src, seg, n):
    return jax.ops.segment_sum(src, seg, n)
class _Rng:
    def __init__(self, key):
        self._k = key
    def _next(self):
        self._k, sub = jax.random.split(self._k)
        return sub
    def normal(self, shape):
        return jax.random.normal(self._next(), shape, dtype=jnp.bfloat16)
    def randint(self, lo, hi, shape):
        return jax.random.randint(self._next(), shape, lo, hi, dtype=jnp.int32)
    def uniform(self, shape, lo=0.0, hi=1.0):
        return jax.random.uniform(self._next(), shape, jnp.bfloat16, lo, hi)
    def permutation(self, n):
        return jax.random.permutation(self._next(), n)


kernel_name = 'gated_mix__grouped_kv_mqa__glu_gated_reglu__prompt'

def setup_inputs():
    _rng = _Rng(jax.random.key(int.from_bytes(__import__("os").urandom(4), "little")))
    _w = (lambda a: (lambda t: t.astype(jnp.bfloat16) if jnp.issubdtype(t.dtype, jnp.floating) else t)(jnp.asarray(a)))
    def _A_setup():
        B, S, D, H = 1, 2048, 640, 32
        Dh = D // H
        return {
            "x": _w((lambda *s: _rng.normal(s) * 0.05)(B, S, D)),
            "wq": _w((lambda *s: _rng.normal(s) * 0.2)(D, H * Dh)),
            "wk": _w((lambda *s: _rng.normal(s) * 0.2)(D, Dh)),
            "wv": _w((lambda *s: _rng.normal(s) * 0.05)(D, Dh)),
            "wo": _w((lambda *s: _rng.normal(s) * 0.05)(H * Dh, D)),
        }
    _A_in = _A_setup()

    def _B_setup():
        B, S, D, F = 1, 2048, 640, 1536
        return {
            "x": _w((lambda *s: _rng.normal(s) * 0.05)(B, S, D)),
            "W_gate": _w((lambda *s: _rng.normal(s) * 0.4)(D, F) * (2.0 / D) ** 0.5),
            "W_up": _w((lambda *s: _rng.normal(s) * 0.4)(D, F) * (2.0 / D) ** 0.5),
            "W_down": _w((lambda *s: _rng.normal(s) * 0.4)(F, D) * (1.0 / F) ** 0.5),
        }
    _B_in = _B_setup()

    return {
        "A_x": _A_in["x"],
        "A_wq": _A_in["wq"],
        "A_wk": _A_in["wk"],
        "A_wv": _A_in["wv"],
        "A_wo": _A_in["wo"],
        "B_x": _B_in["x"],
        "B_W_gate": _B_in["W_gate"],
        "B_W_up": _B_in["W_up"],
        "B_W_down": _B_in["W_down"],
        "gate_w": _w((lambda *s: _rng.normal(s) * 0.05)(640) * 16.0),
    }

def reference(A_x, A_wq, A_wk, A_wv, A_wo, B_x, B_W_gate, B_W_up, B_W_down, gate_w):
    def _A_ref(x, wq, wk, wv, wo):
        B, S, D = x.shape
        H = 32
        Dh = D // H
        q = (lambda x, *d: x.transpose(*d))((x @ wq).reshape(B, S, H, Dh), 0, 2, 1, 3)
        k = x @ wk
        v = x @ wv
        scores = jnp.einsum("bhqd,bkd->bhqk", q, k) * (Dh ** -0.5)
        p = _softmax(scores, axis=-1)
        o = jnp.einsum("bhqk,bkd->bhqd", p, v)
        return (lambda x, *d: x.transpose(*d))(o, 0, 2, 1, 3).reshape(B, S, H * Dh) @ wo

    def _B_ref(x, W_gate, W_up, W_down):
        gate = jnp.einsum("bsd,df->bsf", x, W_gate)
        up = jnp.einsum("bsd,df->bsf", x, W_up)
        gate = gate * (lambda x, dt: x.astype(dt))(gate > 0, gate.dtype)
        h = gate * up
        return jnp.einsum("bsf,fd->bsd", h, W_down)

    x = A_x
    g = _sigmoid((x * gate_w).sum(-1, keepdims=True))
    a = _A_ref(x, A_wq, A_wk, A_wv, A_wo)
    b = _B_ref(x, B_W_gate, B_W_up, B_W_down)
    return g * a + (1 - g) * b
```

```python
import functools
import math

import jax
import jax.numpy as jnp
from jax import lax
import jax.experimental.pallas as pl
import jax.experimental.pallas.tpu as pltpu

F32 = jnp.float32
BF16 = jnp.bfloat16

TQ = 512
HG = 8
KC = 128
LAG1 = 2
LAG2 = 1
FC = 512
VROWS = 24

_NT = (((1,), (1,)), ((), ()))
_NN = (((1,), (0,)), ((), ()))
_TN = (((0,), (0,)), ((), ()))


def _kernel(x_ref, wq_ref, wkt_ref, wvt_ref, gw_ref, wo_hbm, wg_hbm, wu_hbm, wd_hbm,
            o_ref,
            k_s, vt_s, wqt_s, qt_s, ot_s, wo_s, wg_s, wu_s, wd_s, sems,
            *, S, D, H, Dh, F):
    i = pl.program_id(0)
    qscale = (Dh ** -0.5) * math.log2(math.e)
    nc = S // KC

    def weight_copies():
        return [
            pltpu.make_async_copy(wo_hbm, wo_s, sems.at[0]),
            pltpu.make_async_copy(wg_hbm, wg_s, sems.at[1]),
            pltpu.make_async_copy(wu_hbm, wu_s, sems.at[2]),
            pltpu.make_async_copy(wd_hbm, wd_s, sems.at[3]),
        ]

    @pl.when(i == 0)
    def _prologue():
        for cp in weight_copies():
            cp.start()
        x = x_ref[...]
        k_s[...] = lax.dot_general(x, wkt_ref[...], _NT,
                                   preferred_element_type=F32).astype(BF16)
        vt = lax.dot_general(wvt_ref[...], x, _NT, preferred_element_type=F32)
        vt_s[0:Dh, :] = vt.astype(BF16).astype(F32)
        row = lax.broadcasted_iota(jnp.int32, (VROWS - Dh, S), 0)
        vt_s[Dh:VROWS, :] = jnp.where(row == 0, 1.0, 0.0).astype(F32)
        wqt_s[...] = wq_ref[...].T

    q0 = pl.multiple_of(i * TQ, TQ)
    xb = x_ref[pl.ds(q0, TQ), :]
    qt = lax.dot_general(wqt_s[...], xb, _NT, preferred_element_type=F32)
    qt_s[...] = (qt * qscale).astype(BF16).reshape(H // HG, HG * Dh, TQ)

    def unit(j, carry):
        qt_all = qt_s[j]
        accs = [None] * HG
        ms = [None] * HG
        pend1 = []
        pend2 = []

        def do_exp(item):
            hh, c, s, mc = item
            m_old = ms[hh]
            m_new = mc if m_old is None else jnp.maximum(m_old, mc)
            ms[hh] = m_new
            alpha = None if m_old is None else jnp.exp2(m_old - m_new)
            p = jnp.exp2(s - m_new).astype(BF16)
            pend2.append((hh, c, p, alpha))

        def do_pv(item):
            hh, c, p, alpha = item
            pv = lax.dot_general(vt_s[:, c * KC:(c + 1) * KC], p, _NN,
                                 preferred_element_type=F32)
            accs[hh] = pv if accs[hh] is None else accs[hh] * alpha + pv
            if c == nc - 1:
                acc = accs[hh]
                ot_s[j, hh * Dh:(hh + 1) * Dh, :] = acc[0:Dh, :] * (1.0 / acc[Dh:Dh + 1, :])

        for hh in range(HG):
            qth = qt_all[hh * Dh:(hh + 1) * Dh, :]
            for c in range(nc):
                s = jnp.dot(k_s[c * KC:(c + 1) * KC, :], qth, preferred_element_type=F32)
                mc = jnp.max(s, axis=0, keepdims=True)
                pend1.append((hh, c, s, mc))
                if len(pend1) > LAG1:
                    do_exp(pend1.pop(0))
                if len(pend2) > LAG2:
                    do_pv(pend2.pop(0))
        while pend1:
            do_exp(pend1.pop(0))
            if len(pend2) > LAG2:
                do_pv(pend2.pop(0))
        while pend2:
            do_pv(pend2.pop(0))
        return carry

    lax.fori_loop(0, H // HG, unit, 0)

    @pl.when(i == 0)
    def _wait_weights():
        for cp in weight_copies():
            cp.wait()

    a = lax.dot_general(ot_s[...].reshape(H * Dh, TQ).astype(BF16), wo_s[...], _TN,
                        preferred_element_type=F32)
    b = None
    for f in range(F // FC):
        gate = jnp.dot(xb, wg_s[:, f * FC:(f + 1) * FC], preferred_element_type=F32)
        up = jnp.dot(xb, wu_s[:, f * FC:(f + 1) * FC], preferred_element_type=F32)
        hmid = (jnp.maximum(gate, 0.0) * up).astype(BF16)
        d = jnp.dot(hmid, wd_s[f * FC:(f + 1) * FC, :], preferred_element_type=F32)
        b = d if b is None else b + d
    logit = jnp.sum(xb.astype(F32) * gw_ref[...].astype(F32), axis=1, keepdims=True)
    g = jax.nn.sigmoid(logit)
    o_ref[...] = (g * a + (1.0 - g) * b).astype(o_ref.dtype)


@jax.jit
def pallas_gated_mix__grouped_kv_mqa__glu_gated_reglu__prompt_kernel(
    A_x: jax.Array,
    A_wq: jax.Array,
    A_wk: jax.Array,
    A_wv: jax.Array,
    A_wo: jax.Array,
    B_x: jax.Array,
    B_W_gate: jax.Array,
    B_W_up: jax.Array,
    B_W_down: jax.Array,
    gate_w: jax.Array,
):
    B, S, D = A_x.shape
    Dh = A_wk.shape[1]
    H = A_wq.shape[1] // Dh
    F = B_W_gate.shape[1]
    x2 = A_x.reshape(S, D)
    gw2 = gate_w.reshape(1, D)

    full = lambda shape: pl.BlockSpec(shape, lambda i: (0, 0))
    hbm = pl.BlockSpec(memory_space=pl.ANY)
    out = pl.pallas_call(
        functools.partial(_kernel, S=S, D=D, H=H, Dh=Dh, F=F),
        grid=(S // TQ,),
        in_specs=[full((S, D)), full((D, H * Dh)), full((Dh, D)), full((Dh, D)), full((1, D)),
                  hbm, hbm, hbm, hbm],
        out_specs=pl.BlockSpec((TQ, D), lambda i: (i, 0)),
        out_shape=jax.ShapeDtypeStruct((S, D), A_x.dtype),
        scratch_shapes=[
            pltpu.VMEM((S, Dh), BF16),
            pltpu.VMEM((VROWS, S), F32),
            pltpu.VMEM((H * Dh, D), BF16),
            pltpu.VMEM((H // HG, HG * Dh, TQ), BF16),
            pltpu.VMEM((H // HG, HG * Dh, TQ), F32),
            pltpu.VMEM((H * Dh, D), BF16),
            pltpu.VMEM((D, F), BF16),
            pltpu.VMEM((D, F), BF16),
            pltpu.VMEM((F, D), BF16),
            pltpu.SemaphoreType.DMA((4,)),
        ],
        compiler_params=pltpu.CompilerParams(
            dimension_semantics=("arbitrary",),
            vmem_limit_bytes=100 * 1024 * 1024),
    )(x2, A_wq, A_wk.T, A_wv.T, gw2, A_wo, B_W_gate, B_W_up, B_W_down)
    return out.reshape(B, S, D)
```

```python
import functools
import math

import jax
import jax.numpy as jnp
from jax import lax
import jax.experimental.pallas as pl
import jax.experimental.pallas.tpu as pltpu

F32 = jnp.float32
BF16 = jnp.bfloat16

TQ = 128
GH = 4
KC = 128
LAG1 = 2
LAG2 = 1
FC = 512
XC = 512
VROWS = 24

_NT = (((1,), (1,)), ((), ()))
_NN = (((1,), (0,)), ((), ()))
_TN = (((0,), (0,)), ((), ()))


def _kernel(x_hbm, wq_hbm, wkt_hbm, wvt_hbm, gw_hbm, wo_hbm, wg_hbm, wu_hbm, wd_hbm,
            o_ref,
            x_s, wq_s, wkt_s, wvt_s, gw_s, wall_s, t0_s, k_s, vt_s, qt_s, ot_s,
            wo_s, wg_s, wu_s, wd_s, sems,
            *, S, D, H, Dh, F):
    i = pl.program_id(0)
    qscale = (Dh ** -0.5) * math.log2(math.e)
    nc = S // KC
    ng = H // GH
    nxc = S // XC
    krow = H * Dh
    vrow = krow + 24
    wrows = krow + 48

    def small_copies():
        return [pltpu.make_async_copy(wkt_hbm, wkt_s, sems.at[0]),
                pltpu.make_async_copy(wvt_hbm, wvt_s, sems.at[1]),
                pltpu.make_async_copy(wq_hbm, wq_s, sems.at[2])]

    def x_copy(c):
        return pltpu.make_async_copy(x_hbm.at[pl.ds(c * XC, XC)], x_s.at[pl.ds(c * XC, XC)],
                                     sems.at[3 + c])

    def weight_copies():
        b = 3 + nxc
        return [pltpu.make_async_copy(wg_hbm, wg_s, sems.at[b]),
                pltpu.make_async_copy(wu_hbm, wu_s, sems.at[b + 1]),
                pltpu.make_async_copy(wd_hbm, wd_s, sems.at[b + 2]),
                pltpu.make_async_copy(wo_hbm, wo_s, sems.at[b + 3]),
                pltpu.make_async_copy(gw_hbm, gw_s, sems.at[b + 4])]

    def prologue():
        for cp in small_copies():
            cp.start()
        for c in range(nxc):
            x_copy(c).start()
        for cp in small_copies():
            cp.wait()
        wall_s[0:krow, :] = wq_s[...].T
        wall_s[krow:wrows, :] = jnp.zeros((wrows - krow, D), BF16)
        wall_s[krow:krow + Dh, :] = wkt_s[...]
        wall_s[vrow:vrow + Dh, :] = wvt_s[...]
        row = lax.broadcasted_iota(jnp.int32, (VROWS - Dh, S), 0)
        vt_s[Dh:VROWS, :] = jnp.where(row == 0, 1.0, 0.0).astype(F32)
        def project(c):
            xc = x_s[c * XC:(c + 1) * XC, :]
            return lax.dot_general(wall_s[...], xc, _NT, preferred_element_type=F32)

        def scatter(c, t):
            qt = (t[0:krow, :] * qscale).astype(BF16)
            for r in range(XC // TQ):
                for g in range(ng):
                    qt_s[c * (XC // TQ) + r, g] = jnp.concatenate(
                        [qt[(g * GH + hh) * Dh:(g * GH + hh + 1) * Dh, r * TQ:(r + 1) * TQ]
                         for hh in range(GH)], axis=1)
            kt = t[krow:krow + 24, :]
            k_s[c * XC:(c + 1) * XC, :] = kt.T[:, 0:Dh].astype(BF16)
            vt_s[0:Dh, c * XC:(c + 1) * XC] = t[vrow:vrow + Dh, :].astype(BF16).astype(F32)

        x_copy(0).wait()
        t0_s[...] = project(0)
        for c in range(1, nxc):
            x_copy(c).wait()
        for cp in weight_copies():
            cp.start()
        scatter(0, t0_s[...])
        for c in range(1, nxc):
            scatter(c, project(c))

    def block(blk, with_attn, with_tail):
        r0 = blk * TQ if isinstance(blk, int) else pl.multiple_of(blk * TQ, TQ)
        st = {}

        def ffn_piece(t):
            f, kind = t // 3, t % 3
            xb = x_s[pl.ds(r0, TQ), :]
            if kind == 0:
                st["g"] = jnp.dot(xb, wg_s[:, f * FC:(f + 1) * FC], preferred_element_type=F32)
            elif kind == 1:
                up = jnp.dot(xb, wu_s[:, f * FC:(f + 1) * FC], preferred_element_type=F32)
                st["h"] = (jnp.maximum(st["g"], 0.0) * up).astype(BF16)
            else:
                d = jnp.dot(st["h"], wd_s[f * FC:(f + 1) * FC, :], preferred_element_type=F32)
                st["b"] = d if f == 0 else st["b"] + d

        npieces = 3 * (F // FC)
        total = ng * nc
        ffn_at = {}
        if with_attn and with_tail:
            for t in range(npieces - 1):
                ffn_at[(t * (total - 1)) // (npieces - 2)] = t

        if with_attn:
            accs = [None] * ng
            ms = [None] * ng
            pend1 = []
            pend2 = []

            def do_exp(item):
                g, c, s, mc = item
                m_old = ms[g]
                m_new = mc if m_old is None else jnp.maximum(m_old, mc)
                ms[g] = m_new
                alpha = None if m_old is None else jnp.exp2(m_old - m_new)
                p = jnp.exp2(s - m_new).astype(BF16)
                pend2.append((g, c, p, alpha))

            def do_pv(item):
                g, c, p, alpha = item
                pv = lax.dot_general(vt_s[:, c * KC:(c + 1) * KC], p, _NN,
                                     preferred_element_type=F32)
                accs[g] = pv if accs[g] is None else accs[g] * alpha + pv
                if c == nc - 1:
                    acc = accs[g]
                    o = acc[0:Dh, :] * (1.0 / acc[Dh:Dh + 1, :])
                    for hh in range(GH):
                        h = g * GH + hh
                        ot_s[h * Dh:(h + 1) * Dh, :] = o[:, hh * TQ:(hh + 1) * TQ]

            n = 0
            for g in range(ng):
                qth = qt_s[blk, g]
                for c in range(nc):
                    s = jnp.dot(k_s[c * KC:(c + 1) * KC, :], qth, preferred_element_type=F32)
                    mc = jnp.max(s, axis=0, keepdims=True)
                    pend1.append((g, c, s, mc))
                    if len(pend1) > LAG1:
                        do_exp(pend1.pop(0))
                    if len(pend2) > LAG2:
                        do_pv(pend2.pop(0))
                    if n in ffn_at:
                        ffn_piece(ffn_at[n])
                    n += 1
            while pend1:
                do_exp(pend1.pop(0))
                if len(pend2) > LAG2:
                    do_pv(pend2.pop(0))
            while pend2:
                do_pv(pend2.pop(0))

        if with_tail:
            for t in range(0 if not with_attn else npieces - 1, npieces):
                ffn_piece(t)
            a = lax.dot_general(ot_s[...].astype(BF16), wo_s[...], _TN,
                                preferred_element_type=F32)
            xb = x_s[pl.ds(r0, TQ), :]
            logit = jnp.sum(xb.astype(F32) * gw_s[...].astype(F32).reshape(1, D), axis=1, keepdims=True)
            gate = jax.nn.sigmoid(logit)
            o_ref[...] = (gate * a + (1.0 - gate) * st["b"]).astype(o_ref.dtype)

    @pl.when(i == 0)
    def _first():
        prologue()
        block(0, True, False)
        for cp in weight_copies():
            cp.wait()
        block(0, False, True)

    @pl.when(i > 0)
    def _rest():
        block(i, True, True)


@jax.jit
def pallas_gated_mix__grouped_kv_mqa__glu_gated_reglu__prompt_kernel(
    A_x: jax.Array,
    A_wq: jax.Array,
    A_wk: jax.Array,
    A_wv: jax.Array,
    A_wo: jax.Array,
    B_x: jax.Array,
    B_W_gate: jax.Array,
    B_W_up: jax.Array,
    B_W_down: jax.Array,
    gate_w: jax.Array,
):
    B, S, D = A_x.shape
    Dh = A_wk.shape[1]
    H = A_wq.shape[1] // Dh
    F = B_W_gate.shape[1]
    x2 = A_x.reshape(S, D)

    hbm = pl.BlockSpec(memory_space=pl.ANY)
    nsem = 3 + S // XC + 5
    out = pl.pallas_call(
        functools.partial(_kernel, S=S, D=D, H=H, Dh=Dh, F=F),
        grid=(S // TQ,),
        in_specs=[hbm] * 9,
        out_specs=pl.BlockSpec((TQ, D), lambda i: (i, 0)),
        out_shape=jax.ShapeDtypeStruct((S, D), A_x.dtype),
        scratch_shapes=[
            pltpu.VMEM((S, D), BF16),
            pltpu.VMEM((D, H * Dh), BF16),
            pltpu.VMEM((Dh, D), BF16),
            pltpu.VMEM((Dh, D), BF16),
            pltpu.VMEM((D,), BF16),
            pltpu.VMEM((H * Dh + 48, D), BF16),
            pltpu.VMEM((H * Dh + 48, XC), F32),
            pltpu.VMEM((S, Dh), BF16),
            pltpu.VMEM((VROWS, S), F32),
            pltpu.VMEM((S // TQ, H // GH, Dh, GH * TQ), BF16),
            pltpu.VMEM((H * Dh, TQ), F32),
            pltpu.VMEM((H * Dh, D), BF16),
            pltpu.VMEM((D, F), BF16),
            pltpu.VMEM((D, F), BF16),
            pltpu.VMEM((F, D), BF16),
            pltpu.SemaphoreType.DMA((nsem,)),
        ],
        compiler_params=pltpu.CompilerParams(
            dimension_semantics=("arbitrary",),
            vmem_limit_bytes=100 * 1024 * 1024),
    )(x2, A_wq, A_wk.T, A_wv.T, gate_w, A_wo, B_W_gate, B_W_up, B_W_down)
    return out.reshape(B, S, D)
```

```python
import functools
import math

import jax
import jax.numpy as jnp
from jax import lax
import jax.experimental.pallas as pl
import jax.experimental.pallas.tpu as pltpu

F32 = jnp.float32
BF16 = jnp.bfloat16

TQ = 128
GH = 4
KC = 128
LAG1 = 1
LAG2 = 1
XC = 512
PADH = 24

_NT = (((1,), (1,)), ((), ()))
_NN = (((1,), (0,)), ((), ()))


def _kernel(x_hbm, wq_hbm, wkt_hbm, wvt_hbm, gw_hbm, wo_hbm, wg_hbm, wu_hbm, wd_hbm,
            o_ref,
            x_s, wq_s, wkt_s, wvt_s, gw_s, wall_s, t0_s, k_s, vt_s, qt_s, ot_s,
            wo_s, wg_s, wu_s, wd_s, sems,
            *, S, D, H, Dh):
    i = pl.program_id(0)
    qscale = (Dh ** -0.5) * math.log2(math.e)
    nc = S // KC
    ng = H // GH
    nxc = S // XC
    krow = H * Dh
    vrow = krow + PADH
    wrows = krow + 2 * PADH

    def qkv_weight_copies():
        return [pltpu.make_async_copy(wkt_hbm, wkt_s, sems.at[0]),
                pltpu.make_async_copy(wvt_hbm, wvt_s, sems.at[1]),
                pltpu.make_async_copy(wq_hbm, wq_s, sems.at[2])]

    def x_copy(c):
        return pltpu.make_async_copy(x_hbm.at[pl.ds(c * XC, XC)], x_s.at[pl.ds(c * XC, XC)],
                                     sems.at[3 + c])

    def tail_weight_copies():
        b = 3 + nxc
        return [pltpu.make_async_copy(wg_hbm, wg_s, sems.at[b]),
                pltpu.make_async_copy(wu_hbm, wu_s, sems.at[b + 1]),
                pltpu.make_async_copy(wd_hbm, wd_s, sems.at[b + 2]),
                pltpu.make_async_copy(wo_hbm, wo_s, sems.at[b + 3]),
                pltpu.make_async_copy(gw_hbm, gw_s, sems.at[b + 4])]

    def prologue():
        for cp in qkv_weight_copies():
            cp.start()
        for c in range(nxc):
            x_copy(c).start()
        for cp in qkv_weight_copies():
            cp.wait()
        wall_s[0:krow, :] = wq_s[...].T
        wall_s[krow:wrows, :] = jnp.zeros((wrows - krow, D), BF16)
        wall_s[krow:krow + Dh, :] = wkt_s[...]
        wall_s[vrow:vrow + Dh, :] = wvt_s[...]
        row = lax.broadcasted_iota(jnp.int32, (PADH - Dh, S), 0)
        vt_s[Dh:PADH, :] = jnp.where(row == 0, 1.0, 0.0).astype(F32)

        def project(c):
            xc = x_s[c * XC:(c + 1) * XC, :]
            return lax.dot_general(wall_s[...], xc, _NT, preferred_element_type=F32)

        def scatter(c, t):
            qt = (t[0:krow, :] * qscale).astype(BF16)
            for r in range(XC // TQ):
                for g in range(ng):
                    qt_s[c * (XC // TQ) + r, g] = jnp.concatenate(
                        [qt[(g * GH + hh) * Dh:(g * GH + hh + 1) * Dh, r * TQ:(r + 1) * TQ]
                         for hh in range(GH)], axis=1)
            kt = t[krow:vrow, :]
            k_s[c * XC:(c + 1) * XC, :] = kt.T[:, 0:Dh].astype(BF16)
            vt_s[0:Dh, c * XC:(c + 1) * XC] = t[vrow:vrow + Dh, :].astype(BF16).astype(F32)

        x_copy(0).wait()
        t0_s[...] = project(0)
        for c in range(1, nxc):
            x_copy(c).wait()
        for cp in tail_weight_copies():
            cp.start()
        scatter(0, t0_s[...])
        for c in range(1, nxc):
            scatter(c, project(c))

    def block(blk, with_attn, with_tail):
        r0 = blk * TQ if isinstance(blk, int) else pl.multiple_of(blk * TQ, TQ)
        ffn = {}

        def ffn_gate():
            ffn["gate"] = jnp.dot(x_s[pl.ds(r0, TQ), :], wg_s[...], preferred_element_type=F32)

        def ffn_up():
            up = jnp.dot(x_s[pl.ds(r0, TQ), :], wu_s[...], preferred_element_type=F32)
            ffn["h"] = (jnp.maximum(ffn["gate"], 0.0) * up).astype(BF16)

        if with_attn:
            total = ng * nc
            ffn_at = {0: ffn_gate, total - 1: ffn_up} if with_tail else {}
            accs = [None] * ng
            ms = [None] * ng
            pend_exp = []
            pend_pv = []

            def do_exp():
                g, c, s, mc = pend_exp.pop(0)
                m_old = ms[g]
                m_new = mc if m_old is None else jnp.maximum(m_old, mc)
                ms[g] = m_new
                alpha = None if m_old is None else jnp.exp2(m_old - m_new)
                p = jnp.exp2(s - m_new).astype(BF16)
                pend_pv.append((g, c, p, alpha))

            def do_pv():
                g, c, p, alpha = pend_pv.pop(0)
                pv = lax.dot_general(vt_s[:, c * KC:(c + 1) * KC], p, _NN,
                                     preferred_element_type=F32)
                accs[g] = pv if accs[g] is None else accs[g] * alpha + pv
                if c == nc - 1:
                    acc = accs[g]
                    o = acc[0:Dh, :] * (1.0 / acc[Dh:Dh + 1, :])
                    for hh in range(GH):
                        h = g * GH + hh
                        ot_s[h * Dh:(h + 1) * Dh, :] = o[:, hh * TQ:(hh + 1) * TQ]

            for g in range(ng):
                qth = qt_s[blk, g]
                for c in range(nc):
                    s = jnp.dot(k_s[c * KC:(c + 1) * KC, :], qth, preferred_element_type=F32)
                    pend_exp.append((g, c, s, jnp.max(s, axis=0, keepdims=True)))
                    if len(pend_exp) > LAG1:
                        do_exp()
                    if len(pend_pv) > LAG2:
                        do_pv()
                    if g * nc + c in ffn_at:
                        ffn_at[g * nc + c]()
            while pend_exp:
                do_exp()
                if len(pend_pv) > LAG2:
                    do_pv()
            while pend_pv:
                do_pv()

        if with_tail:
            if not with_attn:
                ffn_gate()
                ffn_up()
            b = jnp.dot(ffn["h"], wd_s[...], preferred_element_type=F32)
            o = ot_s[...].astype(BF16).T
            nl = D - 128
            kl = H * Dh - 128
            a_lo = jnp.dot(o, wo_s[:, 0:nl], preferred_element_type=F32)
            a_hi = jnp.dot(o[:, 0:kl], wo_s[0:kl, nl:D], preferred_element_type=F32)
            qr = TQ // 4
            a_hi = a_hi + jnp.concatenate(
                [jnp.dot(o[r * qr:(r + 1) * qr, kl:], wo_s[kl:, nl:D], preferred_element_type=F32)
                 for r in range(4)], axis=0)
            a = jnp.concatenate([a_lo, a_hi], axis=1)
            xb = x_s[pl.ds(r0, TQ), :]
            logit = jnp.sum(xb.astype(F32) * gw_s[...].astype(F32).reshape(1, D),
                            axis=1, keepdims=True)
            gate = jax.nn.sigmoid(logit)
            o_ref[...] = (gate * a + (1.0 - gate) * b).astype(o_ref.dtype)

    @pl.when(i == 0)
    def _first():
        prologue()
        block(0, True, False)
        for cp in tail_weight_copies():
            cp.wait()
        block(0, False, True)

    @pl.when(i > 0)
    def _rest():
        block(i, True, True)


@jax.jit
def pallas_gated_mix__grouped_kv_mqa__glu_gated_reglu__prompt_kernel(
    A_x: jax.Array,
    A_wq: jax.Array,
    A_wk: jax.Array,
    A_wv: jax.Array,
    A_wo: jax.Array,
    B_x: jax.Array,
    B_W_gate: jax.Array,
    B_W_up: jax.Array,
    B_W_down: jax.Array,
    gate_w: jax.Array,
):
    B, S, D = A_x.shape
    Dh = A_wk.shape[1]
    H = A_wq.shape[1] // Dh
    F = B_W_gate.shape[1]
    assert B == 1 and S % XC == 0 and H % GH == 0 and Dh < PADH and D % 128 == 0

    hbm = pl.BlockSpec(memory_space=pl.ANY)
    out = pl.pallas_call(
        functools.partial(_kernel, S=S, D=D, H=H, Dh=Dh),
        grid=(S // TQ,),
        in_specs=[hbm] * 9,
        out_specs=pl.BlockSpec((TQ, D), lambda i: (i, 0)),
        out_shape=jax.ShapeDtypeStruct((S, D), A_x.dtype),
        scratch_shapes=[
            pltpu.VMEM((S, D), BF16),
            pltpu.VMEM((D, H * Dh), BF16),
            pltpu.VMEM((Dh, D), BF16),
            pltpu.VMEM((Dh, D), BF16),
            pltpu.VMEM((D,), BF16),
            pltpu.VMEM((H * Dh + 2 * PADH, D), BF16),
            pltpu.VMEM((H * Dh + 2 * PADH, XC), F32),
            pltpu.VMEM((S, Dh), BF16),
            pltpu.VMEM((PADH, S), F32),
            pltpu.VMEM((S // TQ, H // GH, Dh, GH * TQ), BF16),
            pltpu.VMEM((H * Dh, TQ), F32),
            pltpu.VMEM((H * Dh, D), BF16),
            pltpu.VMEM((D, F), BF16),
            pltpu.VMEM((D, F), BF16),
            pltpu.VMEM((F, D), BF16),
            pltpu.SemaphoreType.DMA((3 + S // XC + 5,)),
        ],
        compiler_params=pltpu.CompilerParams(
            dimension_semantics=("arbitrary",),
            vmem_limit_bytes=100 * 1024 * 1024),
    )(A_x.reshape(S, D), A_wq, A_wk.T, A_wv.T, gate_w, A_wo, B_W_gate, B_W_up, B_W_down)
    return out.reshape(B, S, D)
```
